```python
import os as _os
_os.environ.setdefault("JAX_PLATFORMS", "cpu")
import jax
import jax.numpy as jnp

def _softmax(x, axis=-1):
    return jax.nn.softmax(x, axis=axis)
def _gelu(x):
    return jax.nn.gelu(x, approximate=True)
def _silu(x):
    return jax.nn.silu(x)
def _sigmoid(x):
    return jax.nn.sigmoid(x)
def _layernorm(x, axis=-1, eps=1e-5):
    m = jnp.mean(x, axis=axis, keepdims=True)
    v = jnp.var(x, axis=axis, keepdims=True)
    return (x - m) / jnp.sqrt(v + eps)
def _scatter_add(tgt, idx, src, axis=0):
    return tgt.at[idx].add(src)
def _segment_sum(src, seg, n):
    return jax.ops.segment_sum(src, seg, n)
class _Rng:
    def __init__(self, key):
        self._k = key
    def _next(self):
        self._k, sub = jax.random.split(self._k)
        return sub
    def normal(self, shape):
        return jax.random.normal(self._next(), shape, dtype=jnp.bfloat16)
    def randint(self, lo, hi, shape):
        return jax.random.randint(self._next(), shape, lo, hi, dtype=jnp.int32)
    def uniform(self, shape, lo=0.0, hi=1.0):
        return jax.random.uniform(self._next(), shape, jnp.bfloat16, lo, hi)
    def permutation(self, n):
        return jax.random.permutation(self._next(), n)


kernel_name = 'parallel_sum__linear_kernel_hedgehog__dense_activation_gelu__prompt'

def setup_inputs():
    _rng = _Rng(jax.random.key(int.from_bytes(__import__("os").urandom(4), "little")))
    _w = (lambda a: (lambda t: t.astype(jnp.bfloat16) if jnp.issubdtype(t.dtype, jnp.floating) else t)(jnp.asarray(a)))
    def _A_setup():
        B, S, D, H = 1, 2048, 448, 16
        Dh = D // H
        return {
            "x": _w((lambda *s: _rng.normal(s) * 0.05)(B, S, D)),
            "wqkv": _w((lambda *s: _rng.normal(s) * 0.2)(D, 3 * D)),
            "w_phi": _w((lambda *s: _rng.normal(s) * 0.2)(H, Dh, Dh) * (Dh ** -0.5)),
            "wo": _w((lambda *s: _rng.normal(s) * 0.05)(D, D)),
        }
    _A_in = _A_setup()

    def _B_setup():
        B, S, D, F = 1, 2048, 448, 1792
        return {
            "x": _w((lambda *s: _rng.normal(s) * 0.05)(B, S, D)),
            "w1": _w((lambda *s: _rng.normal(s) * 0.2)(D, F) * (D ** -0.5)),
            "b1": _w((lambda *s: _rng.normal(s) * 0.2)(F) * 0.01),
            "w2": _w((lambda *s: _rng.normal(s) * 0.2)(F, D) * (F ** -0.5)),
            "b2": _w((lambda *s: _rng.normal(s) * 0.05)(D) * 0.01),
        }
    _B_in = _B_setup()

    return {
        "A_x": _A_in["x"],
        "A_wqkv": _A_in["wqkv"],
        "A_w_phi": _A_in["w_phi"],
        "A_wo": _A_in["wo"],
        "B_x": _B_in["x"],
        "B_w1": _B_in["w1"],
        "B_b1": _B_in["b1"],
        "B_w2": _B_in["w2"],
        "B_b2": _B_in["b2"],
    }

def reference(A_x, A_wqkv, A_w_phi, A_wo, B_x, B_w1, B_b1, B_w2, B_b2):
    def _A_ref(x, wqkv, w_phi, wo):
        B, S, D = x.shape
        H = 16; Dh = D // H
        qkv = (lambda x, *d: x.transpose(*d))((x @ wqkv).reshape(B, S, 3, H, Dh), 2, 0, 3, 1, 4)
        q, k, v = qkv[0], qkv[1], qkv[2]
        pq = jnp.einsum("bhsd,hdf->bhsf", q, w_phi)
        pk = jnp.einsum("bhsd,hdf->bhsf", k, w_phi)
        phi_q = jnp.concatenate([_softmax(pq, axis=-1), _softmax(-pq, axis=-1)], axis=-1)
        phi_k = jnp.concatenate([_softmax(pk, axis=-1), _softmax(-pk, axis=-1)], axis=-1)
        kv = jnp.einsum("bhsf,bhsd->bhfd", phi_k, v)
        z  = jnp.einsum("bhsf->bhf", phi_k)
        num = jnp.einsum("bhqf,bhfd->bhqd", phi_q, kv)
        den = jnp.einsum("bhqf,bhf->bhq", phi_q, z)[..., None] + 1e-6
        o = num / den
        return (lambda x, *d: x.transpose(*d))(o, 0, 2, 1, 3).reshape(B, S, D) @ wo

    def _B_ref(x, w1, b1, w2, b2):
        h = jnp.einsum("bsd,df->bsf", x, w1) + b1
        h = _gelu(h)
        return jnp.einsum("bsf,fd->bsd", h, w2) + b2

    x = A_x
    xn = _layernorm(x, axis=-1)
    return x + _A_ref(xn, A_wqkv, A_w_phi, A_wo) + _B_ref(xn, B_w1, B_b1, B_w2, B_b2)
```

```python
import functools

import jax
import jax.numpy as jnp
from jax import lax
import jax.experimental.pallas as pl
import jax.experimental.pallas.tpu as pltpu

_H = 16
_G = 4
_TS = 512
_NT = (((1,), (1,)), ((), ()))
_TN = (((0,), (0,)), ((), ()))
_F32 = jnp.float32
_BF16 = jnp.bfloat16


def _dot(a, b, dims=(((1,), (0,)), ((), ()))):
    return lax.dot_general(a, b, dims, preferred_element_type=_F32)


def _iota(shape, d):
    return lax.broadcasted_iota(jnp.int32, shape, d)


def _dual_softmax(p, dh):
    t = p.shape[1]
    p3 = p.reshape(dh // 2, 8, t)

    def full(r, op):
        return op(r, pltpu.roll(r, 4, 0))

    mx = full(jnp.max(p3, axis=0), jnp.maximum)
    mn = full(jnp.min(p3, axis=0), jnp.minimum)
    ep = jnp.exp(p3 - mx[None])
    en = jnp.exp(mn[None] - p3)
    rp = 1.0 / full(jnp.sum(ep, axis=0), jnp.add)
    rn = 1.0 / full(jnp.sum(en, axis=0), jnp.add)
    ep = (ep * rp[None]).reshape(dh * _G, t).astype(_BF16)
    en = (en * rn[None]).reshape(dh * _G, t).astype(_BF16)
    return jnp.concatenate([ep, en], axis=0)


def _kernel(x_hbm, wqkv_hbm, wphi_ref, wo_hbm, w1_hbm, b1_ref, w2_hbm, b2_ref,
            out_hbm,
            x_v, xn_v, wqkv_v, wo_v, w1_v, w2_v, out_v, wphi2_v, wT_v, wop_v,
            kv_v, sem_x, sem_w, sem_o, *, S, D, F):
    dh = D // _H
    gw = dh * _G
    ng = _H // _G
    nt = S // _TS

    def x_copy(i):
        return pltpu.make_async_copy(x_hbm.at[0, pl.ds(i * _TS, _TS)],
                                     x_v.at[pl.ds(i * _TS, _TS)], sem_x.at[i])

    def o_copy(i):
        return pltpu.make_async_copy(out_v.at[pl.ds(i * _TS, _TS)],
                                     out_hbm.at[0, pl.ds(i * _TS, _TS)],
                                     sem_o.at[i])

    c_qkv = pltpu.make_async_copy(wqkv_hbm, wqkv_v, sem_w.at[0])
    c_wo = pltpu.make_async_copy(wo_hbm, wo_v, sem_w.at[1])
    c_w1 = pltpu.make_async_copy(w1_hbm, w1_v, sem_w.at[2])
    c_w2 = pltpu.make_async_copy(w2_hbm, w2_v, sem_w.at[3])
    c_qkv.start()
    for i in range(nt):
        x_copy(i).start()
    c_wo.start()
    c_w1.start()
    c_w2.start()

    pad = 64
    wphi2_v[0:pad, :] = jnp.zeros((pad, dh), _F32)
    wphi2_v[pad + D:2 * pad + D, :] = jnp.zeros((pad, dh), _F32)
    for h in range(_H):
        wphi2_v[pad + h * dh:pad + (h + 1) * dh, :] = wphi_ref[h].astype(_F32)

    r_e = _iota((gw, dh), 0)
    emat = ((r_e >> 2) == _iota((gw, dh), 1)).astype(_F32).astype(_BF16)

    def windows(width, off, start):
        row = _iota((gw, width), 0)
        col = _iota((gw, width), 1) + (start - off)
        return row, col

    c_qkv.wait()
    for part in range(3):
        base = part * D
        for g in range(ng):
            lo = base + g * gw
            start = (lo // 128) * 128
            width = min(-(-(lo + gw) // 128) * 128, 3 * D) - start
            row, col = windows(width, lo, start)
            rhs = wqkv_v[:, start:start + width]
            hrow = (row & 3) * dh
            if part < 2:
                n = -(-width // 8) * 8
                s0 = pad + g * gw - (lo - start)
                s1 = (s0 // 8) * 8
                wp = wphi2_v[s1:s1 + n + 8, :]
                wp = wp[s0 - s1:s0 - s1 + width].astype(_BF16)
                sel = _dot(emat, wp, _NT)
                lhs = jnp.where((col >= hrow) & (col < hrow + dh), sel, 0.0)
            else:
                lhs = (col == hrow + (row >> 2)).astype(_F32)
            wt = _dot(lhs.astype(_BF16), rhs, _NT)
            wT_v[base + g * gw:base + (g + 1) * gw, :] = wt.astype(_BF16)

    ones = jnp.ones((128 - gw, _TS), _BF16)

    for g in range(ng):
        kv_v[g] = jnp.zeros((128, 2 * gw), _F32)

    def phase1(i, carry):
        x_copy(i).wait()
        rows = pl.ds(pl.multiple_of(i * _TS, _TS), _TS)
        x = x_v[rows, :].astype(_F32)
        mu = jnp.mean(x, axis=-1, keepdims=True)
        xc = x - mu
        var = jnp.mean(xc * xc, axis=-1, keepdims=True)
        xn = (xc * lax.rsqrt(var + 1e-5)).astype(_BF16)
        xn_v[rows, :] = xn
        kvt = _dot(wT_v[D:3 * D, :], xn, _NT)
        for g in range(ng):
            phi = _dual_softmax(kvt[g * gw:(g + 1) * gw], dh)
            vt = kvt[D + g * gw:D + (g + 1) * gw].astype(_BF16)
            vt = jnp.concatenate([vt, ones], axis=0)
            kv_v[g] += _dot(vt, phi, _NT)
        return carry

    lax.fori_loop(0, nt, phase1, 0)

    for g in range(ng):
        same = (_iota((128, 2 * gw), 0) & 3) == (_iota((128, 2 * gw), 1) & 3)
        kv_v[g] = jnp.where(same, kv_v[g], 0.0)

    c_wo.wait()
    row = _iota((D, D), 0)
    col = _iota((D, D), 1)
    grp = row // gw
    rin = row - grp * gw
    perm = (col == grp * gw + (rin & 3) * dh + (rin >> 2))
    wop_v[...] = _dot(perm.astype(_F32).astype(_BF16), wo_v[...]).astype(_BF16)
    c_w1.wait()
    c_w2.wait()

    def phase2(i, carry):
        rows = pl.ds(pl.multiple_of(i * _TS, _TS), _TS)
        xn = xn_v[rows, :]
        qt = _dot(wT_v[0:D, :], xn, _NT)
        outs = []
        for g in range(ng):
            phi = _dual_softmax(qt[g * gw:(g + 1) * gw], dh)
            nd = _dot(kv_v[g].astype(_BF16), phi)
            inv = 1.0 / (nd[gw:gw + 8] + 1e-6)
            o = nd[0:gw].reshape(dh // 2, 8, _TS) * inv[None]
            outs.append(o.reshape(gw, _TS).astype(_BF16))
        ot = jnp.concatenate(outs, axis=0)
        acc = _dot(ot, wop_v[...], _TN)
        h = _dot(xn, w1_v[...]) + b1_ref[...].astype(_F32)
        h = jax.nn.gelu(h, approximate=True).astype(_BF16)
        acc = acc + _dot(h, w2_v[...])
        acc = acc + (x_v[rows, :].astype(_F32) + b2_ref[...].astype(_F32))
        out_v[rows, :] = acc.astype(_BF16)
        o_copy(i).start()
        return carry

    lax.fori_loop(0, nt, phase2, 0)
    for i in range(nt):
        o_copy(i).wait()


@jax.jit
def pallas_parallel_sum__linear_kernel_hedgehog__dense_activation_gelu__prompt_kernel(
    A_x: jax.Array,
    A_wqkv: jax.Array,
    A_w_phi: jax.Array,
    A_wo: jax.Array,
    B_x: jax.Array,
    B_w1: jax.Array,
    B_b1: jax.Array,
    B_w2: jax.Array,
    B_b2: jax.Array,
):
    del B_x
    _, S, D = A_x.shape
    F = B_w1.shape[1]
    dh = D // _H
    nt = S // _TS
    hbm = pl.BlockSpec(memory_space=pl.ANY)
    vmem = pl.BlockSpec(memory_space=pltpu.VMEM)
    return pl.pallas_call(
        functools.partial(_kernel, S=S, D=D, F=F),
        out_shape=jax.ShapeDtypeStruct(A_x.shape, A_x.dtype),
        in_specs=[hbm, hbm, vmem, hbm, hbm, vmem, hbm, vmem],
        out_specs=hbm,
        scratch_shapes=[
            pltpu.VMEM((S, D), _BF16),
            pltpu.VMEM((S, D), _BF16),
            pltpu.VMEM((D, 3 * D), _BF16),
            pltpu.VMEM((D, D), _BF16),
            pltpu.VMEM((D, F), _BF16),
            pltpu.VMEM((F, D), _BF16),
            pltpu.VMEM((S, D), _BF16),
            pltpu.VMEM((D + 128 + 256, dh), _F32),
            pltpu.VMEM((3 * D, D), _BF16),
            pltpu.VMEM((D, D), _BF16),
            pltpu.VMEM((_H // _G, 128, 2 * dh * _G), _F32),
            pltpu.SemaphoreType.DMA((nt,)),
            pltpu.SemaphoreType.DMA((4,)),
            pltpu.SemaphoreType.DMA((nt,)),
        ],
        compiler_params=pltpu.CompilerParams(vmem_limit_bytes=100 * 1024 * 1024),
    )(A_x, A_wqkv, A_w_phi, A_wo, B_w1, B_b1.reshape(1, F), B_w2,
      B_b2.reshape(1, D))
```

```python
import functools

import jax
import jax.numpy as jnp
from jax import lax
import jax.experimental.pallas as pl
import jax.experimental.pallas.tpu as pltpu

_H = 16
_G = 4
_TS = 512
_NT = (((1,), (1,)), ((), ()))
_TN = (((0,), (0,)), ((), ()))
_F32 = jnp.float32
_BF16 = jnp.bfloat16


def _dot(a, b, dims=(((1,), (0,)), ((), ()))):
    return lax.dot_general(a, b, dims, preferred_element_type=_F32)


def _iota(shape, d):
    return lax.broadcasted_iota(jnp.int32, shape, d)


def _dual_softmax(p, dh):
    t = p.shape[1]
    p3 = p.reshape(dh // 2, 8, t)

    def full(r, op):
        return op(r, pltpu.roll(r, 4, 0))

    mx = full(jnp.max(p3, axis=0), jnp.maximum)
    mn = full(jnp.min(p3, axis=0), jnp.minimum)
    ep = jnp.exp(p3 - mx[None])
    en = jnp.exp(mn[None] - p3)
    rp = 1.0 / full(jnp.sum(ep, axis=0), jnp.add)
    rn = 1.0 / full(jnp.sum(en, axis=0), jnp.add)
    ep = (ep * rp[None]).reshape(dh * _G, t).astype(_BF16)
    en = (en * rn[None]).reshape(dh * _G, t).astype(_BF16)
    return jnp.concatenate([ep, en], axis=0)


def _kernel(x_hbm, wqkv_hbm, wphi_ref, wo_hbm, w1_hbm, b1_ref, w2_hbm, b2_ref,
            out_hbm,
            x_v, xn_v, wqkv_v, wo_v, w1_v, w1T_v, w2_v, out_v, wphi2_v, wT_v,
            wop_v,
            kv_v, sem_x, sem_w, sem_o, *, S, D, F):
    dh = D // _H
    gw = dh * _G
    ng = _H // _G
    nt = S // _TS

    def x_copy(i):
        return pltpu.make_async_copy(x_hbm.at[0, :, pl.ds(i * _TS, _TS)],
                                     x_v.at[:, pl.ds(i * _TS, _TS)], sem_x.at[i])

    def o_copy(i):
        return pltpu.make_async_copy(out_v.at[:, pl.ds(i * _TS, _TS)],
                                     out_hbm.at[0, :, pl.ds(i * _TS, _TS)],
                                     sem_o.at[i])

    c_qkv = pltpu.make_async_copy(wqkv_hbm, wqkv_v, sem_w.at[0])
    c_wo = pltpu.make_async_copy(wo_hbm, wo_v, sem_w.at[1])
    c_w1 = pltpu.make_async_copy(w1_hbm, w1_v.at[0:D], sem_w.at[2])
    c_w2 = pltpu.make_async_copy(w2_hbm, w2_v, sem_w.at[3])
    c_qkv.start()
    for i in range(nt):
        x_copy(i).start()
    c_wo.start()
    c_w1.start()
    c_w2.start()

    pad = 64
    nr = wphi2_v.shape[0]
    r = _iota((nr, D), 0) - pad
    c = _iota((nr, D), 1)
    pm = (r == (c & (_H - 1)) * dh + (c >> 4)).astype(_F32).astype(_BF16)
    wphi2_v[...] = _dot(pm, wphi_ref[...].reshape(D, dh))

    r_e = _iota((gw, dh), 0)
    emat = ((r_e >> 2) == _iota((gw, dh), 1)).astype(_F32).astype(_BF16)

    def windows(width, off, start):
        row = _iota((gw, width), 0)
        col = _iota((gw, width), 1) + (start - off)
        return row, col

    c_qkv.wait()
    for part in range(3):
        base = part * D
        for g in range(ng):
            lo = base + g * gw
            start = (lo // 128) * 128
            width = min(-(-(lo + gw) // 128) * 128, 3 * D) - start
            row, col = windows(width, lo, start)
            rhs = wqkv_v[:, start:start + width]
            hrow = (row & 3) * dh
            if part < 2:
                n = -(-width // 8) * 8
                s0 = pad + g * gw - (lo - start)
                s1 = (s0 // 8) * 8
                wp = wphi2_v[s1:s1 + n + 8, :]
                wp = wp[s0 - s1:s0 - s1 + width].astype(_BF16)
                sel = _dot(emat, wp, _NT)
                lhs = jnp.where((col >= hrow) & (col < hrow + dh), sel, 0.0)
            else:
                lhs = (col == hrow + (row >> 2)).astype(_F32)
            wt = _dot(lhs.astype(_BF16), rhs, _NT)
            wT_v[base + g * gw:base + (g + 1) * gw, :] = wt.astype(_BF16)

    ones = jnp.ones((128 - gw, _TS), _BF16)

    kp = xn_v.shape[0] - D
    xn_v[D:, :] = (_iota((kp, S), 0) == 0).astype(_F32).astype(_BF16)

    def bias_rows(b_ref):
        n = b_ref.shape[0]
        b = jnp.broadcast_to(b_ref[...].astype(_F32).reshape(1, n), (kp, n))
        return jnp.where(_iota((kp, n), 0) == 0, b, 0.0)

    for g in range(ng):
        kv_v[g] = jnp.zeros((128, 2 * gw), _F32)

    def phase1(i, carry):
        x_copy(i).wait()
        rows = pl.ds(pl.multiple_of(i * _TS, _TS), _TS)
        x = x_v[:, rows].astype(_F32)
        mu = jnp.mean(x, axis=0, keepdims=True)
        xc = x - mu
        var = jnp.mean(xc * xc, axis=0, keepdims=True)
        xn = (xc * lax.rsqrt(var + 1e-5)).astype(_BF16)
        xn_v[0:D, rows] = xn
        kvt = _dot(wT_v[D:3 * D, :], xn)
        for g in range(ng):
            phi = _dual_softmax(kvt[g * gw:(g + 1) * gw], dh)
            vt = kvt[D + g * gw:D + (g + 1) * gw].astype(_BF16)
            vt = jnp.concatenate([vt, ones], axis=0)
            kv_v[g] += _dot(vt, phi, _NT)
        return carry

    for i in range(nt):
        phase1(i, 0)

    for g in range(ng):
        same = (_iota((128, 2 * gw), 0) & 3) == (_iota((128, 2 * gw), 1) & 3)
        kv_v[g] = jnp.where(same, kv_v[g], 0.0)

    c_wo.wait()
    row = _iota((D, D), 0)
    col = _iota((D, D), 1)
    grp = sum((row >= g * gw).astype(jnp.int32) for g in range(1, ng))
    rin = row - grp * gw
    perm = (col == grp * gw + (rin & 3) * dh + (rin >> 2))
    wop = _dot(perm.astype(_F32).astype(_BF16), wo_v[...])
    wop_v[...] = jnp.concatenate([wop, bias_rows(b2_ref)], axis=0).T.astype(_BF16)
    c_w1.wait()
    w1_v[D:, :] = bias_rows(b1_ref).astype(_BF16)
    w1T_v[...] = w1_v[...].T
    c_w2.wait()

    def phase2(i, carry):
        rows = pl.ds(pl.multiple_of(i * _TS, _TS), _TS)
        xn = xn_v[:, rows]
        qt = _dot(wT_v[0:D, :], xn[0:D])
        outs = []
        for g in range(ng):
            phi = _dual_softmax(qt[g * gw:(g + 1) * gw], dh)
            nd = _dot(kv_v[g].astype(_BF16), phi)
            inv = 1.0 / (nd[gw:gw + 8] + 1e-6)
            o = nd[0:gw].reshape(dh // 2, 8, _TS) * inv[None]
            outs.append(o.reshape(gw, _TS).astype(_BF16))
        ot = jnp.concatenate(outs + [xn[D:]], axis=0)
        acc = _dot(wop_v[...], ot)
        h = _dot(w1T_v[...], xn)
        h = jax.nn.gelu(h, approximate=True).astype(_BF16)
        acc = acc + _dot(w2_v[...], h)
        acc = acc + x_v[:, rows].astype(_F32)
        out_v[:, rows] = acc.astype(_BF16)
        o_copy(i).start()
        return carry

    lax.fori_loop(0, nt, phase2, 0)
    for i in range(nt):
        o_copy(i).wait()


@jax.jit
def pallas_parallel_sum__linear_kernel_hedgehog__dense_activation_gelu__prompt_kernel(
    A_x: jax.Array,
    A_wqkv: jax.Array,
    A_w_phi: jax.Array,
    A_wo: jax.Array,
    B_x: jax.Array,
    B_w1: jax.Array,
    B_b1: jax.Array,
    B_w2: jax.Array,
    B_b2: jax.Array,
):
    del B_x
    _, S, D = A_x.shape
    F = B_w1.shape[1]
    dh = D // _H
    nt = S // _TS
    hbm = pl.BlockSpec(memory_space=pltpu.HBM)
    vmem = pl.BlockSpec(memory_space=pltpu.VMEM)
    KP = -(-(D + 1) // 128) * 128
    out_t = pl.pallas_call(
        functools.partial(_kernel, S=S, D=D, F=F),
        out_shape=jax.ShapeDtypeStruct((1, D, S), A_x.dtype),
        in_specs=[hbm, hbm, vmem, hbm, hbm, vmem, hbm, vmem],
        out_specs=hbm,
        scratch_shapes=[
            pltpu.VMEM((D, S), _BF16),
            pltpu.VMEM((KP, S), _BF16),
            pltpu.VMEM((D, 3 * D), _BF16),
            pltpu.VMEM((D, D), _BF16),
            pltpu.VMEM((KP, F), _BF16),
            pltpu.VMEM((F, KP), _BF16),
            pltpu.VMEM((D, F), _BF16),
            pltpu.VMEM((D, S), _BF16),
            pltpu.VMEM((D + 128 + 256, dh), _F32),
            pltpu.VMEM((3 * D, D), _BF16),
            pltpu.VMEM((D, KP), _BF16),
            pltpu.VMEM((_H // _G, 128, 2 * dh * _G), _F32),
            pltpu.SemaphoreType.DMA((nt,)),
            pltpu.SemaphoreType.DMA((4,)),
            pltpu.SemaphoreType.DMA((nt,)),
        ],
        compiler_params=pltpu.CompilerParams(vmem_limit_bytes=100 * 1024 * 1024),
    )(A_x.transpose(0, 2, 1), A_wqkv, A_w_phi.transpose(1, 0, 2), A_wo, B_w1,
      B_b1, B_w2.T, B_b2)
    return out_t.transpose(0, 2, 1)
```

```python
import functools

import jax
import jax.numpy as jnp
from jax import lax
import jax.experimental.pallas as pl
import jax.experimental.pallas.tpu as pltpu

_H = 16
_G = 4
_TS = 512
_NT = (((1,), (1,)), ((), ()))
_TN = (((0,), (0,)), ((), ()))
_F32 = jnp.float32
_BF16 = jnp.bfloat16


def _dot(a, b, dims=(((1,), (0,)), ((), ()))):
    return lax.dot_general(a, b, dims, preferred_element_type=_F32)


def _iota(shape, d):
    return lax.broadcasted_iota(jnp.int32, shape, d)


def _dual_softmax(p, dh):
    t = p.shape[1]
    p3 = p.reshape(dh // 2, 8, t)

    def full(r, op):
        return op(r, pltpu.roll(r, 4, 0))

    mx = full(jnp.max(p3, axis=0), jnp.maximum)
    mn = full(jnp.min(p3, axis=0), jnp.minimum)
    ep = jnp.exp(p3 - mx[None])
    en = jnp.exp(mn[None] - p3)
    rp = 1.0 / full(jnp.sum(ep, axis=0), jnp.add)
    rn = 1.0 / full(jnp.sum(en, axis=0), jnp.add)
    ep = (ep * rp[None]).reshape(dh * _G, t).astype(_BF16)
    en = (en * rn[None]).reshape(dh * _G, t).astype(_BF16)
    return jnp.concatenate([ep, en], axis=0)


def _kernel(x_hbm, wqkv_hbm, wphi_hbm, wo_hbm, w1_hbm, b1_hbm, w2_hbm, b2_hbm,
            out_hbm,
            x_v, xn_v, wqkv_v, wo_v, w1_v, w1T_v, w2_v, out_v, wphi2_v, wT_v,
            wop_v, wphi_ref, b1_ref, b2_ref,
            kv_v, sem_x, sem_w, sem_o, *, S, D, F):
    dh = D // _H
    gw = dh * _G
    ng = _H // _G
    nt = S // _TS

    def x_copy(i):
        return pltpu.make_async_copy(x_hbm.at[0, :, pl.ds(i * _TS, _TS)],
                                     x_v.at[:, pl.ds(i * _TS, _TS)], sem_x.at[i])

    def o_copy(i):
        return pltpu.make_async_copy(out_v.at[:, pl.ds(i * _TS, _TS)],
                                     out_hbm.at[0, :, pl.ds(i * _TS, _TS)],
                                     sem_o.at[i])

    c_qkv = pltpu.make_async_copy(wqkv_hbm, wqkv_v, sem_w.at[0])
    c_wo = pltpu.make_async_copy(wo_hbm, wo_v, sem_w.at[1])
    c_w1 = pltpu.make_async_copy(w1_hbm, w1_v.at[0:D], sem_w.at[2])
    c_w2 = pltpu.make_async_copy(w2_hbm, w2_v, sem_w.at[3])
    c_ph = pltpu.make_async_copy(wphi_hbm, wphi_ref, sem_w.at[4])
    c_b1 = pltpu.make_async_copy(b1_hbm, b1_ref, sem_w.at[5])
    c_b2 = pltpu.make_async_copy(b2_hbm, b2_ref, sem_w.at[6])
    c_ph.start()
    c_qkv.start()
    x_copy(0).start()

    pad = 64
    nr = wphi2_v.shape[0]
    r = _iota((nr, D), 0) - pad
    c = _iota((nr, D), 1)
    pm = (r == (c & (_H - 1)) * dh + (c >> 4)).astype(_F32).astype(_BF16)
    c_ph.wait()
    wphi2_v[...] = _dot(pm, wphi_ref[...].reshape(D, dh))

    r_e = _iota((gw, dh), 0)
    emat = ((r_e >> 2) == _iota((gw, dh), 1)).astype(_F32).astype(_BF16)

    def windows(width, off, start):
        row = _iota((gw, width), 0)
        col = _iota((gw, width), 1) + (start - off)
        return row, col

    c_qkv.wait()
    for i in range(1, nt):
        x_copy(i).start()
    c_wo.start()
    c_w1.start()
    c_w2.start()
    c_b1.start()
    c_b2.start()
    def fold(part):
        base = part * D
        for g in range(ng):
            lo = base + g * gw
            start = (lo // 128) * 128
            width = min(-(-(lo + gw) // 128) * 128, 3 * D) - start
            row, col = windows(width, lo, start)
            rhs = wqkv_v[:, start:start + width]
            hrow = (row & 3) * dh
            if part < 2:
                n = -(-width // 8) * 8
                s0 = pad + g * gw - (lo - start)
                s1 = (s0 // 8) * 8
                wp = wphi2_v[s1:s1 + n + 8, :]
                wp = wp[s0 - s1:s0 - s1 + width].astype(_BF16)
                sel = _dot(emat, wp, _NT)
                lhs = jnp.where((col >= hrow) & (col < hrow + dh), sel, 0.0)
            else:
                lhs = (col == hrow + (row >> 2)).astype(_F32)
            wt = _dot(lhs.astype(_BF16), rhs, _NT)
            wT_v[base + g * gw:base + (g + 1) * gw, :] = wt.astype(_BF16)

    fold(1)
    fold(2)
    ones = jnp.ones((128 - gw, _TS), _BF16)

    kp = xn_v.shape[0] - D
    xn_v[D:, :] = (_iota((kp, S), 0) == 0).astype(_F32).astype(_BF16)

    def bias_rows(b_ref):
        n = b_ref.shape[0]
        b = jnp.broadcast_to(b_ref[...].astype(_F32).reshape(1, n), (kp, n))
        return jnp.where(_iota((kp, n), 0) == 0, b, 0.0)

    for g in range(ng):
        kv_v[g] = jnp.zeros((128, 2 * gw), _F32)

    def phase1(i, carry):
        x_copy(i).wait()
        rows = pl.ds(pl.multiple_of(i * _TS, _TS), _TS)
        x = x_v[:, rows].astype(_F32)
        mu = jnp.mean(x, axis=0, keepdims=True)
        xc = x - mu
        var = jnp.mean(xc * xc, axis=0, keepdims=True)
        xn = (xc * lax.rsqrt(var + 1e-5)).astype(_BF16)
        xn_v[0:D, rows] = xn
        kvt = _dot(wT_v[D:3 * D, :], xn)
        for g in range(ng):
            phi = _dual_softmax(kvt[g * gw:(g + 1) * gw], dh)
            vt = kvt[D + g * gw:D + (g + 1) * gw].astype(_BF16)
            vt = jnp.concatenate([vt, ones], axis=0)
            kv_v[g] += _dot(vt, phi, _NT)
        return carry

    for i in range(nt):
        phase1(i, 0)

    for g in range(ng):
        same = (_iota((128, 2 * gw), 0) & 3) == (_iota((128, 2 * gw), 1) & 3)
        kv_v[g] = jnp.where(same, kv_v[g], 0.0)

    fold(0)
    c_wo.wait()
    c_b1.wait()
    c_b2.wait()
    parts = []
    for g in range(ng):
        lo = g * gw
        start = (lo // 128) * 128
        width = min(-(-(lo + gw) // 128) * 128, D) - start
        row, col = windows(width, lo, start)
        perm = (col == (row & 3) * dh + (row >> 2)).astype(_F32).astype(_BF16)
        parts.append(_dot(perm, wo_v[start:start + width, :]))
    wop_v[...] = jnp.concatenate(parts + [bias_rows(b2_ref)], axis=0).T.astype(_BF16)
    c_w1.wait()
    w1_v[D:, :] = bias_rows(b1_ref).astype(_BF16)
    w1T_v[...] = w1_v[...].T
    c_w2.wait()

    def phase2(i, carry):
        rows = pl.ds(pl.multiple_of(i * _TS, _TS), _TS)
        xn = xn_v[:, rows]
        qt = _dot(wT_v[0:D, :], xn[0:D])
        outs = []
        for g in range(ng):
            phi = _dual_softmax(qt[g * gw:(g + 1) * gw], dh)
            nd = _dot(kv_v[g].astype(_BF16), phi)
            inv = 1.0 / (nd[gw:gw + 8] + 1e-6)
            o = nd[0:gw].reshape(dh // 2, 8, _TS) * inv[None]
            outs.append(o.reshape(gw, _TS).astype(_BF16))
        ot = jnp.concatenate(outs + [xn[D:]], axis=0)
        acc = _dot(wop_v[...], ot)
        h = _dot(w1T_v[...], xn)
        h = jax.nn.gelu(h, approximate=True).astype(_BF16)
        acc = acc + _dot(w2_v[...], h)
        acc = acc + x_v[:, rows].astype(_F32)
        out_v[:, rows] = acc.astype(_BF16)
        o_copy(i).start()
        return carry

    lax.fori_loop(0, nt, phase2, 0)
    for i in range(nt):
        o_copy(i).wait()


@jax.jit
def pallas_parallel_sum__linear_kernel_hedgehog__dense_activation_gelu__prompt_kernel(
    A_x: jax.Array,
    A_wqkv: jax.Array,
    A_w_phi: jax.Array,
    A_wo: jax.Array,
    B_x: jax.Array,
    B_w1: jax.Array,
    B_b1: jax.Array,
    B_w2: jax.Array,
    B_b2: jax.Array,
):
    del B_x
    _, S, D = A_x.shape
    F = B_w1.shape[1]
    dh = D // _H
    nt = S // _TS
    hbm = pl.BlockSpec(memory_space=pltpu.HBM)
    KP = -(-(D + 1) // 128) * 128
    out_t = pl.pallas_call(
        functools.partial(_kernel, S=S, D=D, F=F),
        out_shape=jax.ShapeDtypeStruct((1, D, S), A_x.dtype),
        in_specs=[hbm] * 8,
        out_specs=hbm,
        scratch_shapes=[
            pltpu.VMEM((D, S), _BF16),
            pltpu.VMEM((KP, S), _BF16),
            pltpu.VMEM((D, 3 * D), _BF16),
            pltpu.VMEM((D, D), _BF16),
            pltpu.VMEM((KP, F), _BF16),
            pltpu.VMEM((F, KP), _BF16),
            pltpu.VMEM((D, F), _BF16),
            pltpu.VMEM((D, S), _BF16),
            pltpu.VMEM((D + 128 + 256, dh), _F32),
            pltpu.VMEM((3 * D, D), _BF16),
            pltpu.VMEM((D, KP), _BF16),
            pltpu.VMEM((dh, _H, dh), _BF16),
            pltpu.VMEM((F,), _BF16),
            pltpu.VMEM((D,), _BF16),
            pltpu.VMEM((_H // _G, 128, 2 * dh * _G), _F32),
            pltpu.SemaphoreType.DMA((nt,)),
            pltpu.SemaphoreType.DMA((7,)),
            pltpu.SemaphoreType.DMA((nt,)),
        ],
        compiler_params=pltpu.CompilerParams(vmem_limit_bytes=100 * 1024 * 1024),
    )(A_x.transpose(0, 2, 1), A_wqkv, A_w_phi.transpose(1, 0, 2), A_wo, B_w1,
      B_b1, B_w2.T, B_b2)
    return out_t.transpose(0, 2, 1)
```
